```python
import os as _os
_os.environ.setdefault("JAX_PLATFORMS", "cpu")
import jax
import jax.numpy as jnp

def _softmax(x, axis=-1):
    return jax.nn.softmax(x, axis=axis)
def _gelu(x):
    return jax.nn.gelu(x, approximate=True)
def _silu(x):
    return jax.nn.silu(x)
def _sigmoid(x):
    return jax.nn.sigmoid(x)
def _layernorm(x, axis=-1, eps=1e-5):
    m = jnp.mean(x, axis=axis, keepdims=True)
    v = jnp.var(x, axis=axis, keepdims=True)
    return (x - m) / jnp.sqrt(v + eps)
def _scatter_add(tgt, idx, src, axis=0):
    return tgt.at[idx].add(src)
def _segment_sum(src, seg, n):
    return jax.ops.segment_sum(src, seg, n)
class _Rng:
    def __init__(self, key):
        self._k = key
    def _next(self):
        self._k, sub = jax.random.split(self._k)
        return sub
    def normal(self, shape):
        return jax.random.normal(self._next(), shape, dtype=jnp.bfloat16)
    def randint(self, lo, hi, shape):
        return jax.random.randint(self._next(), shape, lo, hi, dtype=jnp.int32)
    def uniform(self, shape, lo=0.0, hi=1.0):
        return jax.random.uniform(self._next(), shape, jnp.bfloat16, lo, hi)
    def permutation(self, n):
        return jax.random.permutation(self._next(), n)


kernel_name = 'standalone__gqa_softmax__near_ridge'

def setup_inputs():
    _rng = _Rng(jax.random.key(int.from_bytes(__import__("os").urandom(4), "little")))
    _w = (lambda a: (lambda t: t.astype(jnp.bfloat16) if jnp.issubdtype(t.dtype, jnp.floating) else t)(jnp.asarray(a)))
    B, Hq, Hkv, Sq, Sk, D = 8, 32, 8, 112, 2048, 128
    return {
        "q": _w((lambda *s: _rng.normal(s) * 0.4)(B, Hq, Sq, D)),
        "k": _w((lambda *s: _rng.normal(s) * 0.4)(B, Hkv, Sk, D)),
        "v": _w((lambda *s: _rng.normal(s) * 0.05)(B, Hkv, Sk, D)),
    }

def reference(q, k, v):
    B, Hq, Sq, D = q.shape
    Hkv = k.shape[1]
    rep = Hq // Hkv
    k = jnp.repeat(k, rep, axis=1)
    v = jnp.repeat(v, rep, axis=1)
    scale = D ** -0.5
    scores = jnp.einsum("bhqd,bhkd->bhqk", q, k) * scale
    p = _softmax(scores, axis=-1)
    return jnp.einsum("bhqk,bhkd->bhqd", p, v)
```

```python
import jax, jax.numpy as jnp, functools
from jax import lax
import jax.experimental.pallas as pl
import jax.experimental.pallas.tpu as pltpu
import math

@jax.jit
def pallas_standalone__gqa_softmax__near_ridge_kernel(q, k, v):
    HB, NA, dpos, nobc, flags, olag, expl, pre = 4, 4, 3, True, None, 4, True, True
    RC, RCS = 64, (80, 80, 80, 80, 64, 64)
    B, Hq, Sq, D = q.shape
    Hkv, Sk = k.shape[1], k.shape[2]
    rep = Hq // Hkv
    M = rep * Sq
    G = B * Hkv
    assert (G - NA) % HB == 0 and NA >= HB
    NS = (G - NA) // HB
    q3 = q.reshape(G, M, D); k3 = k.reshape(G, Sk, D); v3 = v.reshape(G, Sk, D)
    c = (D ** -0.5) * math.log2(math.e)
    RCS = tuple(RCS) if RCS else (RC,) * (M // RC)
    assert sum(RCS) == M
    NC = len(RCS); R0 = [sum(RCS[:i]) for i in range(NC)]; RC = RCS[0]
    KR = NA + 1; VR = NA
    OB = KR + 3 * HB

    def body(q_hbm, k_hbm, v_hbm, o_hbm, qo, kb, vb, sb, aq, ak, av, ao, sq, sk, sv, so):
        qb32 = qo.bitcast(jnp.uint32); kb32 = kb.bitcast(jnp.uint32); vb32 = vb.bitcast(jnp.uint32)
        cp = pltpu.make_async_copy

        def qk(pos, ch, slot):
            qq = pltpu.bitcast(qb32[pos, R0[ch]//2:(R0[ch]+RCS[ch])//2, :], jnp.bfloat16)
            if pre:
                qq = (qq.astype(jnp.float32) * c).astype(jnp.bfloat16)
            kk = pltpu.bitcast(kb32[pos], jnp.bfloat16)
            s = lax.dot_general(qq, kk, (((1,), (1,)), ((), ())), preferred_element_type=jnp.float32)
            m = jnp.max(s, axis=-1, keepdims=True)
            return s, m

        def smpv(pos, s, m):
            p = jnp.exp2(s - m) if pre else jnp.exp2((s - m) * c)
            pb = p.astype(jnp.bfloat16)
            l = jnp.sum(p, axis=-1, keepdims=True)
            vv = pltpu.bitcast(vb32[pos], jnp.bfloat16)
            o = jnp.dot(pb, vv, preferred_element_type=jnp.float32)
            r = pl.reciprocal(l, approx=True)
            r = r * (2.0 - l * r)
            return (o * r).astype(jnp.bfloat16)

        def stream(kpos, vpos, opos, knext, hook, dpos):
            n = len(kpos)
            items = [(hh, ch) for hh in range(n) for ch in range(NC)]
            assert len(items) % 2 == 1 or not expl or True
            s = None; m = sb[1, :, 0:1]
            pend = []
            for i, (hh, ch) in enumerate(items):
                last = i + 1 == len(items)
                sn, mn = qk(knext, 0, 0) if last else qk(kpos[items[i + 1][0]], items[i + 1][1], 0)
                if hook is not None and i == dpos:
                    hook()
                if s is None:
                    s = sb[0]
                o = smpv(vpos[hh], s, m)
                pend.append((hh, ch, o))
                if olag is None or len(pend) > olag:
                    ph, pc, po = pend.pop(0)
                    qo[opos[ph], R0[pc]:R0[pc]+RCS[pc], :] = po
                if last:
                    sb[0] = sn
                    sb[1, :, 0:128] = jnp.broadcast_to(mn, (RC, 128))
                s, m = sn, mn
            for ph, pc, po in pend:
                qo[opos[ph], R0[pc]:R0[pc]+RCS[pc], :] = po

        P0 = NA
        c0q = cp(q_hbm.at[0], qo.at[P0], aq.at[NA]); c0k = cp(k_hbm.at[0], kb.at[P0], ak.at[NA])
        c0q.start(); c0k.start()
        c0q.wait(); c0k.wait()
        def a_q(j): return cp(q_hbm.at[j + 1], qo.at[j], aq.at[j])
        def a_k(j): return cp(k_hbm.at[j + 1], kb.at[j], ak.at[j])
        def a_v(j): return cp(v_hbm.at[j], vb.at[j], av.at[j])
        def a_o(j): return cp(qo.at[OB + j], o_hbm.at[j], ao.at[j])
        a_v(0).start(); a_q(0).start(); a_k(0).start()
        s, m = qk(P0, 0, 0)
        sb[0] = s
        sb[1, :, 0:128] = jnp.broadcast_to(m, (RC, 128))

        def stepA(j, carry):
            a_q(j).wait(); a_k(j).wait(); a_v(j).wait()
            kp = jnp.where(j == 0, P0, j - 1)
            def hook():
                @pl.when(j + 1 < NA)
                def _():
                    a_v(j + 1).start(); a_q(j + 1).start(); a_k(j + 1).start()
                @pl.when(j < HB)
                def _():
                    cp(v_hbm.at[NA + j], vb.at[VR + j], sv.at[0]).start()
                    cp(q_hbm.at[NA + 1 + j], qo.at[KR + j], sq.at[0]).start()
                    cp(k_hbm.at[NA + 1 + j], kb.at[KR + j], sk.at[0]).start()
                @pl.when(j >= 1)
                def _():
                    a_o(j - 1).start()
            stream([kp], [j], [OB + j], j, hook, 0)
            return carry
        lax.fori_loop(0, NA, stepA, 0)

        def cp_kq(ref_hbm, buf, sem, h, slot):
            g0 = NA + h * HB
            ge = jnp.minimum(g0 + HB, G - 1)
            base = KR + slot * HB
            out = []
            if HB > 1:
                out.append(cp(ref_hbm.at[pl.ds(g0 + 1, HB - 1)], buf.at[pl.ds(base, HB - 1)], sem.at[slot]))
            out.append(cp(ref_hbm.at[ge], buf.at[base + HB - 1], sem.at[slot]))
            return out
        def cp_v(h, vs): return cp(v_hbm.at[pl.ds(NA + h * HB, HB)], vb.at[pl.ds(VR + vs * HB, HB)], sv.at[vs])
        def cp_o(h, vs): return cp(qo.at[pl.ds(OB + VR + vs * HB, HB)], o_hbm.at[pl.ds(NA + h * HB, HB)], so.at[vs])
        def stepB(h, carry):
            kfirst, ks, ksn, vs = carry
            kbase = KR + ks * HB
            cp(qo.at[pl.ds(kbase, HB)], qo.at[pl.ds(kbase, HB)], sq.at[ks]).wait()
            cp(kb.at[pl.ds(kbase, HB)], kb.at[pl.ds(kbase, HB)], sk.at[ks]).wait()
            cp_v(h, vs).wait()
            @pl.when(h >= 2)
            def _():
                cp_o(h - 2, vs).wait()
            def hook():
                @pl.when(h + 1 < NS)
                def _():
                    cp_v(h + 1, 1 - vs).start()
                    for x in cp_kq(q_hbm, qo, sq, h + 1, ksn) + cp_kq(k_hbm, kb, sk, h + 1, ksn):
                        x.start()
                @pl.when(h >= 1)
                def _():
                    cp_o(h - 1, 1 - vs).start()
                @pl.when(h == 0)
                def _():
                    a_o(NA - 1).start()
            kpos = [kfirst] + [kbase + i for i in range(HB - 1)]
            vpos = [VR + vs * HB + i for i in range(HB)]
            stream(kpos, vpos, [OB + x for x in vpos], kbase + HB - 1, hook, dpos)
            return (kbase + HB - 1, ksn, 3 - ks - ksn, 1 - vs)
        z = jnp.int32(0)
        lax.fori_loop(0, NS, stepB, (z + NA - 1, z, z + 1, z))
        vl = (NS - 1) % 2
        cp_o(NS - 1, vl).start()
        for j in range(NA):
            a_o(j).wait()
        cp_o(NS - 2, 1 - vl).wait()
        cp_o(NS - 1, vl).wait()

    out = pl.pallas_call(
        body,
        in_specs=[pl.BlockSpec(memory_space=pl.ANY)] * 3,
        out_specs=pl.BlockSpec(memory_space=pl.ANY),
        out_shape=jax.ShapeDtypeStruct((G, M, D), q.dtype),
        scratch_shapes=[pltpu.VMEM((OB + VR + 2 * HB, M, D), jnp.bfloat16), pltpu.VMEM((KR + 3 * HB, Sk, D), jnp.bfloat16),
                        pltpu.VMEM((VR + 2 * HB, Sk, D), jnp.bfloat16),
                        pltpu.VMEM((2, RC, Sk), jnp.float32),
                        pltpu.SemaphoreType.DMA((NA + 1,)), pltpu.SemaphoreType.DMA((NA + 1,)),
                        pltpu.SemaphoreType.DMA((NA,)), pltpu.SemaphoreType.DMA((NA,)),
                        pltpu.SemaphoreType.DMA((3,)), pltpu.SemaphoreType.DMA((3,)),
                        pltpu.SemaphoreType.DMA((2,)), pltpu.SemaphoreType.DMA((2,))],
        compiler_params=pltpu.CompilerParams(vmem_limit_bytes=110 * 1024 * 1024, disable_bounds_checks=nobc, flags=flags),
    )(q3, k3, v3)
    return out.reshape(B, Hq, Sq, D)
```

```python
import math

import jax
import jax.numpy as jnp
from jax import lax
import jax.experimental.pallas as pl
import jax.experimental.pallas.tpu as pltpu

HB = 4
NA = 4
RCS = (80, 80, 80, 80, 64, 64)
OLAG = 4
DPOS = 1


@jax.jit
def pallas_standalone__gqa_softmax__near_ridge_kernel(q, k, v):
    B, Hq, Sq, D = q.shape
    Hkv, Sk = k.shape[1], k.shape[2]
    M = (Hq // Hkv) * Sq
    G = B * Hkv
    assert (G - NA) % HB == 0 and HB == NA and sum(RCS) == M and RCS[0] == max(RCS)
    NS = (G - NA) // HB
    NC = len(RCS)
    R0 = [sum(RCS[:i]) for i in range(NC)]
    RC = RCS[0]
    c = (D ** -0.5) * math.log2(math.e)
    KR, VR = NA + 1, NA
    OB = KR + 3 * HB
    P0 = NA

    def body(q_hbm, k_hbm, v_hbm, o_hbm, qo, kb, vb, sb, aq, ak, av, ao, sq, sk, sv, so):
        qb32 = qo.bitcast(jnp.uint32)
        kb32 = kb.bitcast(jnp.uint32)
        vb32 = vb.bitcast(jnp.uint32)
        cp = pltpu.make_async_copy

        def qk(pos, ch):
            qq = pltpu.bitcast(qb32[pos, R0[ch] // 2:(R0[ch] + RCS[ch]) // 2, :], jnp.bfloat16)
            qq = (qq.astype(jnp.float32) * c).astype(jnp.bfloat16)
            kk = pltpu.bitcast(kb32[pos], jnp.bfloat16)
            s = lax.dot_general(qq, kk, (((1,), (1,)), ((), ())), preferred_element_type=jnp.float32)
            return s, jnp.max(s, axis=-1, keepdims=True)

        def smpv(pos, s, m):
            p = jnp.exp2(s - m)
            l = jnp.sum(p, axis=-1, keepdims=True)
            vv = pltpu.bitcast(vb32[pos], jnp.bfloat16)
            o = jnp.dot(p.astype(jnp.bfloat16), vv, preferred_element_type=jnp.float32)
            r = pl.reciprocal(l, approx=True)
            r = r * (2.0 - l * r)
            return (o * r).astype(jnp.bfloat16)

        def carry_out(s, m):
            sb[0] = s
            sb[1, :, 0:128] = jnp.broadcast_to(m, (RC, 128))

        def stream(kpos, vpos, knext, hook, dpos, ohook=None):
            items = [(hh, ch) for hh in range(len(kpos)) for ch in range(NC)]
            s, m = None, sb[1, :, 0:1]
            pend = []

            def flush():
                ph, pc, po = pend.pop(0)
                qo[OB + vpos[ph], R0[pc]:R0[pc] + RCS[pc], :] = po
                if ohook is not None and pc == NC - 1:
                    ohook(ph)

            for i, (hh, ch) in enumerate(items):
                last = i + 1 == len(items)
                sn, mn = qk(knext, 0) if last else qk(kpos[items[i + 1][0]], items[i + 1][1])
                if i == dpos:
                    hook()
                if s is None:
                    s = sb[0]
                pend.append((hh, ch, smpv(vpos[hh], s, m)))
                if len(pend) > OLAG:
                    flush()
                if last:
                    carry_out(sn, mn)
                s, m = sn, mn
            while pend:
                flush()

        c0q = cp(q_hbm.at[0], qo.at[P0], aq.at[NA])
        c0k = cp(k_hbm.at[0], kb.at[P0], ak.at[NA])
        c0q.start(); c0k.start()
        c0q.wait(); c0k.wait()
        def a_q(j): return cp(q_hbm.at[j + 1], qo.at[j], aq.at[j])
        def a_k(j): return cp(k_hbm.at[j + 1], kb.at[j], ak.at[j])
        def a_v(j): return cp(v_hbm.at[j], vb.at[j], av.at[j])
        def a_o(j): return cp(qo.at[OB + j], o_hbm.at[j], ao.at[j])
        a_v(0).start(); a_q(0).start(); a_k(0).start()
        carry_out(*qk(P0, 0))

        def step_a(j, carry):
            a_q(j).wait(); a_k(j).wait(); a_v(j).wait()

            def hook():
                @pl.when(j + 1 < NA)
                def _():
                    a_v(j + 1).start(); a_q(j + 1).start(); a_k(j + 1).start()
                cp(v_hbm.at[NA + j], vb.at[VR + j], sv.at[0]).start()
                cp(q_hbm.at[NA + 1 + j], qo.at[KR + j], sq.at[0]).start()
                cp(k_hbm.at[NA + 1 + j], kb.at[KR + j], sk.at[0]).start()

                @pl.when(j >= 1)
                def _():
                    a_o(j - 1).start()
            stream([jnp.where(j == 0, P0, j - 1)], [j], j, hook, 0)
            return carry
        lax.fori_loop(0, NA, step_a, 0)

        def start_kq(hbm, buf, sem, h, slot):
            g0 = NA + h * HB
            base = KR + slot * HB
            cp(hbm.at[pl.ds(g0 + 1, HB - 1)], buf.at[pl.ds(base, HB - 1)], sem.at[slot]).start()
            cp(hbm.at[jnp.minimum(g0 + HB, G - 1)], buf.at[base + HB - 1], sem.at[slot]).start()
        def cp_v(h, vs): return cp(v_hbm.at[pl.ds(NA + h * HB, HB)], vb.at[pl.ds(VR + vs * HB, HB)], sv.at[vs])
        def cp_o(h, vs): return cp(qo.at[pl.ds(OB + VR + vs * HB, HB)], o_hbm.at[pl.ds(NA + h * HB, HB)], so.at[vs])

        def step_b(h, carry):
            kfirst, ks, ksn, vs = carry
            kbase = KR + ks * HB
            cp(qo.at[pl.ds(kbase, HB)], qo.at[pl.ds(kbase, HB)], sq.at[ks]).wait()
            cp(kb.at[pl.ds(kbase, HB)], kb.at[pl.ds(kbase, HB)], sk.at[ks]).wait()
            cp_v(h, vs).wait()

            @pl.when(h >= 2)
            def _():
                cp_o(h - 2, vs).wait()

            def hook():
                @pl.when(h + 1 < NS)
                def _():
                    cp_v(h + 1, 1 - vs).start()
                    start_kq(q_hbm, qo, sq, h + 1, ksn)
                    start_kq(k_hbm, kb, sk, h + 1, ksn)

                @pl.when(h == 0)
                def _():
                    a_o(NA - 1).start()
            kpos = [kfirst] + [kbase + i for i in range(HB - 1)]
            vpos = [VR + vs * HB + i for i in range(HB)]

            def ohook(ph):
                cp(qo.at[OB + vpos[ph]], o_hbm.at[NA + h * HB + ph], so.at[vs]).start()
            stream(kpos, vpos, kbase + HB - 1, hook, DPOS, ohook)
            return (kbase + HB - 1, ksn, 3 - ks - ksn, 1 - vs)
        z = jnp.int32(0)
        lax.fori_loop(0, NS, step_b, (z + NA - 1, z, z + 1, z))

        vl = (NS - 1) % 2
        for j in range(NA):
            a_o(j).wait()
        cp_o(NS - 2, 1 - vl).wait()
        cp_o(NS - 1, vl).wait()

    dma = pltpu.SemaphoreType.DMA
    out = pl.pallas_call(
        body,
        in_specs=[pl.BlockSpec(memory_space=pl.ANY)] * 3,
        out_specs=pl.BlockSpec(memory_space=pl.ANY),
        out_shape=jax.ShapeDtypeStruct((G, M, D), q.dtype),
        scratch_shapes=[
            pltpu.VMEM((OB + VR + 2 * HB, M, D), jnp.bfloat16),
            pltpu.VMEM((KR + 3 * HB, Sk, D), jnp.bfloat16),
            pltpu.VMEM((VR + 2 * HB, Sk, D), jnp.bfloat16),
            pltpu.VMEM((2, RC, Sk), jnp.float32),
            dma((NA + 1,)), dma((NA + 1,)), dma((NA,)), dma((NA,)),
            dma((3,)), dma((3,)), dma((2,)), dma((2,)),
        ],
        compiler_params=pltpu.CompilerParams(
            vmem_limit_bytes=110 * 1024 * 1024, disable_bounds_checks=True),
    )(q.reshape(G, M, D), k.reshape(G, Sk, D), v.reshape(G, Sk, D))
    return out.reshape(B, Hq, Sq, D)
```
